```python
import os as _os
_os.environ.setdefault("JAX_PLATFORMS", "cpu")
import jax
import jax.numpy as jnp

def _softmax(x, axis=-1):
    return jax.nn.softmax(x, axis=axis)
def _gelu(x):
    return jax.nn.gelu(x, approximate=True)
def _silu(x):
    return jax.nn.silu(x)
def _sigmoid(x):
    return jax.nn.sigmoid(x)
def _layernorm(x, axis=-1, eps=1e-5):
    m = jnp.mean(x, axis=axis, keepdims=True)
    v = jnp.var(x, axis=axis, keepdims=True)
    return (x - m) / jnp.sqrt(v + eps)
def _scatter_add(tgt, idx, src, axis=0):
    return tgt.at[idx].add(src)
def _segment_sum(src, seg, n):
    return jax.ops.segment_sum(src, seg, n)
class _Rng:
    def __init__(self, key):
        self._k = key
    def _next(self):
        self._k, sub = jax.random.split(self._k)
        return sub
    def normal(self, shape):
        return jax.random.normal(self._next(), shape, dtype=jnp.bfloat16)
    def randint(self, lo, hi, shape):
        return jax.random.randint(self._next(), shape, lo, hi, dtype=jnp.int32)
    def uniform(self, shape, lo=0.0, hi=1.0):
        return jax.random.uniform(self._next(), shape, jnp.bfloat16, lo, hi)
    def permutation(self, n):
        return jax.random.permutation(self._next(), n)


kernel_name = 'sequential_preLN__linear_kernel_hedgehog__glu_gated_swiglu__prompt'

def setup_inputs():
    _rng = _Rng(jax.random.key(int.from_bytes(__import__("os").urandom(4), "little")))
    _w = (lambda a: (lambda t: t.astype(jnp.bfloat16) if jnp.issubdtype(t.dtype, jnp.floating) else t)(jnp.asarray(a)))
    def _A_setup():
        B, S, D, H = 1, 2048, 640, 32
        Dh = D // H
        return {
            "x": _w((lambda *s: _rng.normal(s) * 0.05)(B, S, D)),
            "wqkv": _w((lambda *s: _rng.normal(s) * 0.2)(D, 3 * D)),
            "w_phi": _w((lambda *s: _rng.normal(s) * 0.2)(H, Dh, Dh) * (Dh ** -0.5)),
            "wo": _w((lambda *s: _rng.normal(s) * 0.05)(D, D)),
        }
    _A_in = _A_setup()

    def _B_setup():
        B, S, D, F = 1, 2048, 640, 1536
        return {
            "x": _w((lambda *s: _rng.normal(s) * 0.05)(B, S, D)),
            "w1": _w((lambda *s: _rng.normal(s) * 0.05)(D, F) * (2.0 / D) ** 0.5),
            "w3": _w((lambda *s: _rng.normal(s) * 0.05)(D, F) * (2.0 / D) ** 0.5),
            "w2": _w((lambda *s: _rng.normal(s) * 0.05)(F, D) * (2.0 / F) ** 0.5),
        }
    _B_in = _B_setup()

    return {
        "A_x": _A_in["x"],
        "A_wqkv": _A_in["wqkv"],
        "A_w_phi": _A_in["w_phi"],
        "A_wo": _A_in["wo"],
        "B_x": _B_in["x"],
        "B_w1": _B_in["w1"],
        "B_w3": _B_in["w3"],
        "B_w2": _B_in["w2"],
    }

def reference(A_x, A_wqkv, A_w_phi, A_wo, B_x, B_w1, B_w3, B_w2):
    def _A_ref(x, wqkv, w_phi, wo):
        B, S, D = x.shape
        H = 32; Dh = D // H
        qkv = (lambda x, *d: x.transpose(*d))((x @ wqkv).reshape(B, S, 3, H, Dh), 2, 0, 3, 1, 4)
        q, k, v = qkv[0], qkv[1], qkv[2]
        pq = jnp.einsum("bhsd,hdf->bhsf", q, w_phi)
        pk = jnp.einsum("bhsd,hdf->bhsf", k, w_phi)
        phi_q = jnp.concatenate([_softmax(pq, axis=-1), _softmax(-pq, axis=-1)], axis=-1)
        phi_k = jnp.concatenate([_softmax(pk, axis=-1), _softmax(-pk, axis=-1)], axis=-1)
        kv = jnp.einsum("bhsf,bhsd->bhfd", phi_k, v)
        z  = jnp.einsum("bhsf->bhf", phi_k)
        num = jnp.einsum("bhqf,bhfd->bhqd", phi_q, kv)
        den = jnp.einsum("bhqf,bhf->bhq", phi_q, z)[..., None] + 1e-6
        o = num / den
        return (lambda x, *d: x.transpose(*d))(o, 0, 2, 1, 3).reshape(B, S, D) @ wo

    def _B_ref(x, w1, w3, w2):
        gate = jnp.einsum("bsd,df->bsf", x, w1)
        up = jnp.einsum("bsd,df->bsf", x, w3)
        h = _silu(gate) * up
        out = jnp.einsum("bsf,fd->bsd", h, w2)
        return out

    x = A_x
    h = x + _A_ref(_layernorm(x, axis=-1), A_wqkv, A_w_phi, A_wo)
    h2 = h + _B_ref(_layernorm(h, axis=-1), B_w1, B_w3, B_w2)
    return h2
```

```python
import functools
import jax
import jax.numpy as jnp
from jax import lax
import jax.experimental.pallas as pl
import jax.experimental.pallas.tpu as pltpu

S, D, H, DH, F = 2048, 640, 32, 20, 1536
G = 4
NG = H // G
GR = G * DH
T = 256
NTILE = S // T
XSPLIT = 2
LOG2E = 1.4426950408889634
LN_EPS = 1e-5
BF = jnp.bfloat16
F32 = jnp.float32

NT = (((1,), (1,)), ((), ()))
TN = (((0,), (0,)), ((), ()))


def _dot(a, b):
    return jnp.dot(a, b, preferred_element_type=F32)


def _dot_nt(a, b):
    return lax.dot_general(a, b, NT, preferred_element_type=F32)


def _dot_tn(a, b):
    return lax.dot_general(a, b, TN, preferred_element_type=F32)


def _layernorm(x):
    m = jnp.mean(x, axis=-1, keepdims=True)
    xc = x - m
    v = jnp.mean(xc * xc, axis=-1, keepdims=True)
    return xc * lax.rsqrt(v + LN_EPS)


def _half_swap(a):
    return pltpu.roll(a, 4, 0)


def _feature_exps(p):
    t = p.shape[-1]
    p3 = p.reshape(GR // 8, 8, t)
    mx = jnp.max(p3, axis=0)
    mx = jnp.maximum(mx, _half_swap(mx))
    mn = jnp.min(p3, axis=0)
    mn = jnp.minimum(mn, _half_swap(mn))
    ep = jnp.exp2(p3 - mx[None])
    en = jnp.exp2(mn[None] - p3)
    sp = jnp.sum(ep, axis=0)
    sp = sp + _half_swap(sp)
    sn = jnp.sum(en, axis=0)
    sn = sn + _half_swap(sn)
    return ep, en, sp, sn


def _kernel(x_hbm, wqkv_hbm, wphi_hbm, wo_hbm, w1_hbm, w3_hbm, w2_hbm, out_hbm,
            x_v, wqkv_v, wphi_v, wo_v, w1_v, w3_v, w2_v, obuf, xn_v,
            wkvT, wqT, p2, bd_v, kv_acc, z_acc, kv_bf, z_b, hn_v, hres_v,
            xsem, wsem, osem):

    xa = pltpu.make_async_copy(x_hbm.at[0, pl.ds(0, XSPLIT * T)], x_v.at[pl.ds(0, XSPLIT * T)], xsem.at[0])
    xb = pltpu.make_async_copy(x_hbm.at[0, pl.ds(XSPLIT * T, S - XSPLIT * T)],
                               x_v.at[pl.ds(XSPLIT * T, S - XSPLIT * T)], xsem.at[1])

    def wqkv_copy(j):
        return pltpu.make_async_copy(wqkv_hbm.at[:, pl.ds(j * D, D)], wqkv_v.at[:, pl.ds(j * D, D)], wsem.at[j])

    cp_phi = pltpu.make_async_copy(wphi_hbm, wphi_v, wsem.at[3])
    cp_wo = pltpu.make_async_copy(wo_hbm, wo_v, wsem.at[4])
    cp_w1 = pltpu.make_async_copy(w1_hbm, w1_v, wsem.at[5])
    cp_w3 = pltpu.make_async_copy(w3_hbm, w3_v, wsem.at[6])
    cp_w2 = pltpu.make_async_copy(w2_hbm, w2_v, wsem.at[7])

    cp_phi.start()
    wqkv_copy(1).start()
    xa.start()
    wqkv_copy(2).start()

    p2[...] = jnp.zeros(p2.shape, F32)
    kv_acc[...] = jnp.zeros(kv_acc.shape, F32)
    z_acc[...] = jnp.zeros(z_acc.shape, F32)
    rh = lax.broadcasted_iota(jnp.int32, (128, D), 0) * DH
    ch = lax.broadcasted_iota(jnp.int32, (128, D), 1)
    rep = jnp.where(jnp.logical_and(ch >= rh, ch < rh + DH), 1.0, 0.0).astype(BF)
    cp_phi.wait()
    for d in range(DH):
        p2[pl.ds(d * 24, DH), pl.ds(0, H)] = wphi_v[d].astype(F32)
    xall = _dot(p2[...].astype(BF), rep)
    c24 = lax.broadcasted_iota(jnp.int32, (24, D), 1)
    cmod = c24 - ((c24 * 3277) >> 16) * DH
    bmat = xall[0:24]
    for d in range(1, DH):
        bmat = jnp.where(cmod == d, xall[d * 24:(d + 1) * 24], bmat)
    bmat = jnp.concatenate([bmat, jnp.zeros((8, D), F32)], axis=0).astype(BF)
    r_i = lax.broadcasted_iota(jnp.int32, (GR, 32), 0)
    c_i = lax.broadcasted_iota(jnp.int32, (GR, 32), 1)
    sel = jnp.where((r_i >> 2) == c_i, 1.0, 0.0).astype(BF)
    a_full = _dot(sel, bmat)
    r2 = lax.broadcasted_iota(jnp.int32, (GR, D), 0) & 3
    c2 = lax.broadcasted_iota(jnp.int32, (GR, D), 1)
    for g in range(NG):
        lo = (g * G + r2) * DH
        m = jnp.logical_and(c2 >= lo, c2 < lo + DH)
        bd_v[g] = jnp.where(m, a_full, 0.0).astype(BF)

    def ktiles(g):
        k0 = (g * GR) // 128 * 128
        k1 = -(-((g + 1) * GR) // 128) * 128
        return k0, k1

    def fold(j, g):
        k0, k1 = ktiles(g)
        w = wqkv_v[:, pl.ds(j * D + k0, k1 - k0)]
        return (_dot_nt(bd_v[g, :, pl.ds(k0, k1 - k0)], w) * LOG2E).astype(BF)

    def ln1(i):
        xn_v[pl.ds(i * T, T), :] = _layernorm(x_v[pl.ds(i * T, T), :].astype(F32)).astype(BF)

    wqkv_copy(1).wait()
    xa.wait()
    xb.start()
    for g in range(NG):
        wkvT[pl.ds(g * GR, GR), :] = fold(1, g)
    ln1(0)
    wqkv_copy(2).wait()
    wqkv_copy(0).start()
    cp_wo.start()
    cp_w1.start()
    cp_w3.start()
    cp_w2.start()
    wkvT[pl.ds(D, D), :] = wqkv_v[:, pl.ds(2 * D, D)].T

    def proj(i):
        kv = _dot_nt(wkvT[...], xn_v[pl.ds(i * T, T), :])
        return kv[:D], kv[D:].astype(BF)

    def soft_kv(pk, vT):
        for g in range(NG):
            ep, en, sp, sn = _feature_exps(pk[g * GR:(g + 1) * GR])
            phi = jnp.concatenate([ep * (1.0 / sp)[None], en * (1.0 / sn)[None]], axis=0)
            phi = phi.reshape(2 * GR, T)
            zs = phi[:, 0:128]
            for j in range(1, T // 128):
                zs = zs + phi[:, j * 128:(j + 1) * 128]
            z_acc[g] += zs
            kv_acc[g] += _dot_nt(vT[g * GR:(g + 1) * GR], phi.astype(BF))

    prev = None
    for i in range(NTILE):
        if i + 1 == XSPLIT:
            xb.wait()
        cur = proj(i)
        if i + 1 < NTILE:
            ln1(i + 1)
        if prev is not None:
            soft_kv(*prev)
        prev = cur

    wqkv_copy(0).wait()
    cp_wo.wait()
    cp_w1.wait()
    cp_w3.wait()
    cp_w2.wait()
    for g in range(NG):
        wqT[pl.ds(g * GR, GR), :] = fold(0, g)

    def qproj(row0):
        return _dot_nt(wqT[...], xn_v[pl.ds(row0, T), :])

    def softq_num(pq):
        o_parts = []
        for g in range(NG):
            ep, en, sp, sn = _feature_exps(pq[g * GR:(g + 1) * GR])
            z = z_b[g].reshape(2 * GR // 8, 8, 128)
            z = jnp.concatenate([z] * (T // 128), axis=-1)
            ap = jnp.sum(ep * z[:GR // 8], axis=0)
            ap = ap + _half_swap(ap)
            an = jnp.sum(en * z[GR // 8:], axis=0)
            an = an + _half_swap(an)
            rp = 1.0 / sp
            rn = 1.0 / sn
            rd = 1.0 / (ap * rp + an * rn + 1e-6)
            phi = jnp.concatenate([ep * (rp * rd)[None], en * (rn * rd)[None]], axis=0)
            phi = phi.reshape(2 * GR, T).astype(BF)
            o_parts.append(_dot(kv_bf[g], phi).astype(BF))
        return jnp.concatenate(o_parts, axis=0)

    def wo_ln2(oT, row0, slot):
        hres = x_v[pl.ds(row0, T), :].astype(F32) + _dot_tn(oT, wo_v[...])
        hres_v[slot] = hres
        return _layernorm(hres).astype(BF)

    FH = F // 2

    def gateup(hn, c):
        gate = _dot(hn, w1_v[:, pl.ds(c * FH, FH)])
        up = _dot(hn, w3_v[:, pl.ds(c * FH, FH)])
        return (gate * jax.nn.sigmoid(gate) * up).astype(BF)

    def out_copy(i):
        return pltpu.make_async_copy(obuf.at[pl.ds(i * T, T)], out_hbm.at[0, pl.ds(i * T, T)], osem.at[i])

    def finish(act, i, row0, slot):
        res = hres_v[slot] + _dot(act, w2_v[...])
        obuf[pl.ds(row0, T), :] = res.astype(BF)
        out_copy(i).start()

    pq0 = qproj(0)
    soft_kv(*prev)
    r3 = lax.broadcasted_iota(jnp.int32, (GR, 2 * GR), 0)
    c3 = (lax.broadcasted_iota(jnp.int32, (GR, 2 * GR), 1) & 3) * DH
    m3 = jnp.logical_and(r3 >= c3, r3 < c3 + DH)
    for g in range(NG):
        kv_bf[g] = jnp.where(m3, kv_acc[g], 0.0).astype(BF)
        z_b[g] = jnp.broadcast_to(jnp.sum(z_acc[g], axis=-1, keepdims=True), (2 * GR, 128))
    hn_v[...] = wo_ln2(softq_num(pq0), 0, 0)

    def phase2(i, c):
        row0 = pl.multiple_of(i * T, T)
        row1 = pl.multiple_of(row0 + T, T)
        slot = i % 2
        hn = hn_v[...]
        pq = qproj(row1)
        a0 = gateup(hn, 0)
        oT = softq_num(pq)
        a1 = gateup(hn, 1)
        hn_next = wo_ln2(oT, row1, 1 - slot)
        finish(jnp.concatenate([a0, a1], axis=1), i, row0, slot)
        hn_v[...] = hn_next
        return c

    lax.fori_loop(0, NTILE - 1, phase2, 0)
    last = NTILE - 1
    hn = hn_v[...]
    finish(jnp.concatenate([gateup(hn, 0), gateup(hn, 1)], axis=1), last, last * T, last % 2)
    for i in range(NTILE):
        out_copy(i).wait()


@jax.jit
def pallas_sequential_preLN__linear_kernel_hedgehog__glu_gated_swiglu__prompt_kernel(
    A_x: jax.Array,
    A_wqkv: jax.Array,
    A_w_phi: jax.Array,
    A_wo: jax.Array,
    B_x: jax.Array,
    B_w1: jax.Array,
    B_w3: jax.Array,
    B_w2: jax.Array,
):
    any_spec = pl.BlockSpec(memory_space=pl.ANY)
    wphi_t = jnp.transpose(A_w_phi, (1, 2, 0))
    return pl.pallas_call(
        _kernel,
        out_shape=jax.ShapeDtypeStruct((1, S, D), BF),
        in_specs=[any_spec] * 7,
        out_specs=any_spec,
        scratch_shapes=[
            pltpu.VMEM((S, D), BF),
            pltpu.VMEM((D, 3 * D), BF),
            pltpu.VMEM((DH, DH, H), BF),
            pltpu.VMEM((D, D), BF),
            pltpu.VMEM((D, F), BF),
            pltpu.VMEM((D, F), BF),
            pltpu.VMEM((F, D), BF),
            pltpu.VMEM((S, D), BF),
            pltpu.VMEM((S, D), BF),
            pltpu.VMEM((2 * D, D), BF),
            pltpu.VMEM((D, D), BF),
            pltpu.VMEM((DH * 24, 128), F32),
            pltpu.VMEM((NG, GR, D), BF),
            pltpu.VMEM((NG, GR, 2 * GR), F32),
            pltpu.VMEM((NG, 2 * GR, 128), F32),
            pltpu.VMEM((NG, GR, 2 * GR), BF),
            pltpu.VMEM((NG, 2 * GR, 128), F32),
            pltpu.VMEM((T, D), BF),
            pltpu.VMEM((2, T, D), F32),
            pltpu.SemaphoreType.DMA((2,)),
            pltpu.SemaphoreType.DMA((8,)),
            pltpu.SemaphoreType.DMA((NTILE,)),
        ],
        compiler_params=pltpu.CompilerParams(vmem_limit_bytes=100 * 1024 * 1024),
    )(A_x, A_wqkv, wphi_t, A_wo, B_w1, B_w3, B_w2)
```

```python
import jax
import jax.numpy as jnp
from jax import lax
import jax.experimental.pallas as pl
import jax.experimental.pallas.tpu as pltpu

S, D, H, DH, F = 2048, 640, 32, 20, 1536
NP = H // 2
PR = 2 * DH
PA = PR + 8
PC = 4 * PR
NPC = D // PC
T = 256
NTILE = S // T
LC = 32
C0 = 256
LOG2E = 1.4426950408889634
LN_EPS = 1e-5
BF = jnp.bfloat16
F32 = jnp.float32

NT = (((1,), (1,)), ((), ()))
TN = (((0,), (0,)), ((), ()))


def _dot(a, b):
    return jnp.dot(a, b, preferred_element_type=F32)


def _dot_nt(a, b):
    return lax.dot_general(a, b, NT, preferred_element_type=F32)


def _dot_tn(a, b):
    return lax.dot_general(a, b, TN, preferred_element_type=F32)


def _layernorm(x):
    m = jnp.mean(x, axis=-1, keepdims=True)
    xc = x - m
    v = jnp.mean(xc * xc, axis=-1, keepdims=True)
    return xc * lax.rsqrt(v + LN_EPS)


U32 = jnp.uint32


def _pk(v):
    return pltpu.bitcast(v, U32)


def _upk(v):
    return pltpu.bitcast(v, BF)


def _recip(x):
    r = pl.reciprocal(x, approx=True)
    return r * (2.0 - x * r)


def _sub_reduce(a, op):
    a = op(a, pltpu.roll(a, 4, 0))
    return op(a, pltpu.roll(a, 2, 0))


def _phi(p):
    t = p.shape[-1]
    p3 = p.reshape(PR // 8, 8, t)
    mx = _sub_reduce(jnp.max(p3, axis=0), jnp.maximum)
    mn = _sub_reduce(jnp.min(p3, axis=0), jnp.minimum)
    ep = jnp.exp2(p3 - mx[None])
    en = jnp.exp2(mn[None] - p3)
    sp = _sub_reduce(jnp.sum(ep, axis=0), jnp.add)
    sn = _sub_reduce(jnp.sum(en, axis=0), jnp.add)
    phi = jnp.concatenate([ep * _recip(sp)[None], en * _recip(sn)[None]], axis=0)
    return phi.reshape(2 * PR, t).astype(BF)


def _kernel(x_hbm, wqkv_hbm, wphi_hbm, wo_hbm, w1_hbm, w3_hbm, w2_hbm, out_hbm,
            x_v, wqkv_v, wphi_v, wo_v, w1_v, w3_v, w2_v, obuf, xn_v,
            wkT, wvT, wqT, perm_v, a1, a2, bd_v, kv_acc, kv_bf, pq_v, hn_v, hres_v,
            wsem, osem):

    def x_copy(lo, hi, k):
        return pltpu.make_async_copy(x_hbm.at[0, pl.ds(lo, hi - lo)], x_v.at[pl.ds(lo, hi - lo)], wsem.at[9 + k])

    def w_copy(lo, hi, k):
        return pltpu.make_async_copy(wqkv_hbm.at[:, pl.ds(lo, hi - lo)], wqkv_v.at[:, pl.ds(lo, hi - lo)], wsem.at[k])

    cp_x0 = x_copy(0, T, 0)
    cp_x1 = x_copy(T, 2 * T, 1)
    cp_xr = x_copy(2 * T, 4 * T, 2)
    cp_xs = x_copy(4 * T, S, 3)
    cp_k0 = w_copy(D, D + C0, 0)
    cp_k1 = w_copy(D + C0, 2 * D, 1)
    cp_v = w_copy(2 * D, 3 * D, 2)
    cp_q = w_copy(0, D, 8)
    cp_phi = pltpu.make_async_copy(wphi_hbm, wphi_v, wsem.at[3])
    cp_wo = pltpu.make_async_copy(wo_hbm, wo_v, wsem.at[4])
    cp_w1 = pltpu.make_async_copy(w1_hbm, w1_v, wsem.at[5])
    cp_w3 = pltpu.make_async_copy(w3_hbm, w3_v, wsem.at[6])
    cp_w2 = pltpu.make_async_copy(w2_hbm, w2_v, wsem.at[7])

    for cp in (cp_phi, cp_x0, cp_k0, cp_k1, cp_x1, cp_v, cp_xr, cp_xs, cp_q, cp_wo, cp_w1, cp_w3, cp_w2):
        cp.start()

    rp = lax.broadcasted_iota(jnp.int32, (D, D), 0)
    cp_ = lax.broadcasted_iota(jnp.int32, (D, D), 1)
    perm_v[...] = jnp.where(cp_ == (rp & (H - 1)) * DH + (rp >> 5), 1.0, 0.0).astype(BF)
    cp_phi.wait()
    for d in range(DH):
        a1[:, pl.ds(d * H, H)] = wphi_v[d].astype(F32)
    a1v = a1[...]
    for j in range(D // 128):
        a2[j, pl.ds(0, DH, stride=2), :] = a1v[:, j * 128:(j + 1) * 128]
        a2[j, pl.ds(1, DH, stride=2), :] = a1v[:, j * 128:(j + 1) * 128]
    a2v = jnp.concatenate([a2[j] for j in range(D // 128)], axis=1)
    a_full = _dot(a2v.astype(BF), perm_v[...])
    r2 = lax.broadcasted_iota(jnp.int32, (PR, 128), 0) & 1
    c2 = lax.broadcasted_iota(jnp.int32, (PR, 128), 1)
    for j in range(D // 128):
        blk = a_full[:, j * 128:(j + 1) * 128]
        parts = []
        for g in range(3 * j, 3 * j + 4):
            lo = (2 * g + r2) * DH - j * 128
            parts.append(jnp.where(jnp.logical_and(c2 >= lo, c2 < lo + DH), blk, 0.0))
        bd_v[j] = jnp.concatenate(parts, axis=0).astype(BF)

    def fold_blk(col0, j):
        return _dot_nt(bd_v[j], wqkv_v[:, pl.ds(col0 + j * 128, 128)])

    def fold(dst, col0, js, carry):
        rows = []
        for j in js:
            fj = fold_blk(col0, j)
            head = fj[:PR] if carry is None else fj[:PR] + carry
            n = PC if j == D // 128 - 1 else PC - PR
            rows += [head, fj[PR:n]]
            carry = fj[PC - PR:]
        rows = jnp.concatenate(rows, axis=0)
        dst[pl.ds(js[0] * (PC - PR) // 2, rows.shape[0] // 2), :] = _pk((rows * LOG2E).astype(BF))
        return carry

    def ln1(i, c):
        r0 = i * T + c * LC
        xn_v[pl.ds(r0 // 2, LC // 2), :] = _pk(_layernorm(x_v[pl.ds(r0, LC), :].astype(F32)).astype(BF))

    NLC = T // LC

    def proj(w, lo, n, i):
        return _dot_nt(_upk(w[pl.ds(lo // 2, n // 2), :]), _upk(xn_v[pl.ds(i * T // 2, T // 2), :]))

    ones8 = jnp.ones((8, T), F32)

    def vaug(v):
        return [jnp.concatenate([v[g * PR:(g + 1) * PR], ones8], axis=0).astype(BF) for g in range(v.shape[0] // PR)]

    def phis(p):
        return [_phi(p[g * PR:(g + 1) * PR]) for g in range(p.shape[0] // PR)]

    def kv_update(i, g0, vs, ps):
        for k, (v, p) in enumerate(zip(vs, ps)):
            r = _dot_nt(v, p)
            if i == 0:
                kv_acc[g0 + k] = r
            else:
                kv_acc[g0 + k] += r

    def qpiece(i, q):
        pq_v[i, pl.ds(q * PC, PC), :] = proj(wqT, q * PC, PC, i)

    cp_x0.wait()
    for c in range(NLC):
        ln1(0, c)
    cp_k0.wait()
    carry = fold(wkT, D, (0, 1), None)
    pk0a = proj(wkT, 0, 6 * PR, 0)
    cp_k1.wait()
    fold(wkT, D, (2, 3, 4), carry)
    ph0 = phis(pk0a)
    cp_x1.wait()
    pk0b = proj(wkT, 6 * PR, 6 * PR, 0)
    for c in range(NLC // 2):
        ln1(1, c)
    pk0c = proj(wkT, 12 * PR, 4 * PR, 0)
    for c in range(NLC // 2, NLC):
        ln1(1, c)
    ph0 += phis(pk0b)
    pk1 = [proj(wkT, 0, PC, 1)]
    ph0 += phis(pk0c)
    pk1.append(proj(wkT, PC, PC, 1))
    ph1 = phis(pk1[0])
    cp_v.wait()
    wvT[pl.ds(0, 128), :] = _pk(wqkv_v[:, pl.ds(2 * D, 256)].T)
    pk1.append(proj(wkT, 2 * PC, PC, 1))
    wvT[pl.ds(128, 192), :] = _pk(wqkv_v[:, pl.ds(2 * D + 256, 384)].T)
    ph1 += phis(pk1[1])
    pk1.append(proj(wkT, 3 * PC, PC, 1))
    ph1 += phis(pk1[2])
    pend = None
    for i in range(2):
        ph = ph0 if i == 0 else ph1
        for q in range(NPC):
            if i == 1 and q == 1:
                cp_xr.wait()
            va = vaug(proj(wvT, q * PC, PC, i))
            if i == 0 and q == 0:
                ph1 += phis(pk1[3])
            if pend is not None:
                kv_update(*pend)
            pend = (i, 4 * q, va, ph[4 * q:4 * q + 4])
            if i == 1 and q >= 1:
                for c in range((q - 1) * 3, min(q * 3, NLC)):
                    ln1(2, c)

    qjobs = [(i, q) for i in range(NTILE) for q in range(NPC)]
    NHOLD = 6
    for i in range(2, NTILE):
        if i == 3:
            cp_xs.wait()
            cp_q.wait()
            cp_wo.wait()
            fold(wqT, 0, (0, 1, 2, 3, 4), None)
        for q in range(NPC):
            pk = proj(wkT, q * PC, PC, i)
            kv_update(*pend)
            if i + 1 < NTILE:
                ln1(i + 1, 2 * q)
                ln1(i + 1, 2 * q + 1)
            va = vaug(proj(wvT, q * PC, PC, i))
            pend = (i, 4 * q, va, phis(pk))
            if i >= 3:
                for _ in range(2 if q == 0 else 1):
                    if len(qjobs) > NHOLD:
                        qpiece(*qjobs.pop(0))

    r3 = lax.broadcasted_iota(jnp.int32, (PA, 2 * PR), 0)
    c3 = lax.broadcasted_iota(jnp.int32, (PA, 2 * PR), 1) & 1
    hl3 = jnp.where(r3 < PR, jnp.where(r3 >= DH, 1, 0), jnp.where(r3 >= PR + 4, 1, 0))
    m3 = hl3 == c3
    low = lax.broadcasted_iota(jnp.int32, (8, T), 0) < 4

    def kv_fin(gs):
        for g in gs:
            kv_bf[g] = jnp.where(m3, kv_acc[g], 0.0).astype(BF)

    def num(g, ph):
        o = _dot(kv_bf[g], ph)
        r = _recip(o[PR:] + 1e-6)
        rs = pltpu.roll(r, 4, 0)
        r0 = jnp.where(low, r, rs)
        r1 = jnp.where(low, rs, r)
        return o[:PR] * jnp.concatenate([r0, r0, r, r1, r1], axis=0)

    def wo_res(oT, row0, slot):
        hres_v[slot] = x_v[pl.ds(row0, T), :].astype(F32) + _dot_tn(oT, wo_v[...])

    def ln2(slot, c):
        hn_v[pl.ds(c * LC // 2, LC // 2), :] = _pk(_layernorm(hres_v[slot, pl.ds(c * LC, LC), :]).astype(BF))

    FH = F // 2

    def gateup(hn, c):
        gate = _dot(hn, w1_v[:, pl.ds(c * FH, FH)])
        up = _dot(hn, w3_v[:, pl.ds(c * FH, FH)])
        hg = 0.5 * gate
        return (hg * (1.0 + jnp.tanh(hg)) * up).astype(BF)

    def out_copy(k, lo, n):
        return pltpu.make_async_copy(obuf.at[pl.ds(lo, n)], out_hbm.at[0, pl.ds(lo, n)], osem.at[k])

    phq = phis(pq_v[0, pl.ds(0, 2 * PC), :])
    qpiece(*qjobs.pop(0))
    kv_fin(range(12))
    phq += phis(pq_v[0, pl.ds(2 * PC, 2 * PC), :])
    kv_update(*pend)
    o_parts = [num(g, phq[g]) for g in range(12)]
    kv_fin(range(12, 16))
    qpiece(*qjobs.pop(0))
    o_parts += [num(g, phq[g]) for g in range(12, 16)]
    qpiece(*qjobs.pop(0))
    wo_res(jnp.concatenate(o_parts, axis=0).astype(BF), 0, 0)
    while qjobs:
        qpiece(*qjobs.pop(0))
    for c in range(NLC):
        ln2(0, c)
    cp_w1.wait()
    cp_w3.wait()
    cp_w2.wait()

    def phase2(i, carry):
        row0 = pl.multiple_of(i * T, T)
        row1 = pl.multiple_of(row0 + T, T)
        slot = i % 2
        hn = _upk(hn_v[...])
        a0 = gateup(hn, 0)
        oT = jnp.concatenate([num(g, _phi(pq_v[i + 1, pl.ds(g * PR, PR), :])) for g in range(NP)], axis=0).astype(BF)
        a1_ = gateup(hn, 1)
        wo_res(oT, row1, 1 - slot)
        act = jnp.concatenate([a0, a1_], axis=1)
        for n in range(D // 128):
            res = hres_v[slot, :, pl.ds(n * 128, 128)] + _dot(act, w2_v[:, pl.ds(n * 128, 128)])
            obuf[pl.ds(row0, T), pl.ds(n * 128, 128)] = res.astype(BF)
            for c in range(2 * n, min(2 * n + 2, NLC)):
                ln2(1 - slot, c)
        out_copy(i, row0, T).start()
        return carry

    lax.fori_loop(0, NTILE - 1, phase2, 0)
    last = NTILE - 1
    hn = _upk(hn_v[...])
    act = jnp.concatenate([gateup(hn, 0), gateup(hn, 1)], axis=1)
    tail = ((0, 128), (128, 64), (192, 64))
    for k, (lo, n) in enumerate(tail):
        res = hres_v[last % 2, pl.ds(lo, n), :] + _dot(act[lo:lo + n], w2_v[...])
        obuf[pl.ds(last * T + lo, n), :] = res.astype(BF)
        out_copy(last + k, last * T + lo, n).start()
    for i in range(NTILE - 1):
        out_copy(i, i * T, T).wait()
    for k, (lo, n) in enumerate(tail):
        out_copy(last + k, last * T + lo, n).wait()


@jax.jit
def pallas_sequential_preLN__linear_kernel_hedgehog__glu_gated_swiglu__prompt_kernel(
    A_x: jax.Array,
    A_wqkv: jax.Array,
    A_w_phi: jax.Array,
    A_wo: jax.Array,
    B_x: jax.Array,
    B_w1: jax.Array,
    B_w3: jax.Array,
    B_w2: jax.Array,
):
    any_spec = pl.BlockSpec(memory_space=pl.ANY)
    wphi_t = jnp.transpose(A_w_phi, (1, 2, 0))
    return pl.pallas_call(
        _kernel,
        out_shape=jax.ShapeDtypeStruct((1, S, D), BF),
        in_specs=[any_spec] * 7,
        out_specs=any_spec,
        scratch_shapes=[
            pltpu.VMEM((S, D), BF),
            pltpu.VMEM((D, 3 * D), BF),
            pltpu.VMEM((DH, DH, H), BF),
            pltpu.VMEM((D, D), BF),
            pltpu.VMEM((D, F), BF),
            pltpu.VMEM((D, F), BF),
            pltpu.VMEM((F, D), BF),
            pltpu.VMEM((S, D), BF),
            pltpu.VMEM((S // 2, D), U32),
            pltpu.VMEM((D // 2, D), U32),
            pltpu.VMEM((D // 2, D), U32),
            pltpu.VMEM((D // 2, D), U32),
            pltpu.VMEM((D, D), BF),
            pltpu.VMEM((DH, D), F32),
            pltpu.VMEM((D // 128, PR, 128), F32),
            pltpu.VMEM((D // 128, PC, 128), BF),
            pltpu.VMEM((NP, PA, 2 * PR), F32),
            pltpu.VMEM((NP, PA, 2 * PR), BF),
            pltpu.VMEM((NTILE, D, T), F32),
            pltpu.VMEM((T // 2, D), U32),
            pltpu.VMEM((2, T, D), F32),
            pltpu.SemaphoreType.DMA((13,)),
            pltpu.SemaphoreType.DMA((NTILE + 2,)),
        ],
        compiler_params=pltpu.CompilerParams(vmem_limit_bytes=100 * 1024 * 1024),
    )(A_x, A_wqkv, wphi_t, A_wo, B_w1, B_w3, B_w2)
```

```python
import jax
import jax.numpy as jnp
from jax import lax
import jax.experimental.pallas as pl
import jax.experimental.pallas.tpu as pltpu

S, D, H, DH, F = 2048, 640, 32, 20, 1536
NP = H // 2
PR = 2 * DH
PA = PR + 8
PC = 4 * PR
NPC = D // PC
T = 256
NTILE = S // T
LC = 32
C0 = 256
LOG2E = 1.4426950408889634
LN_EPS = 1e-5
BF = jnp.bfloat16
F32 = jnp.float32

NT = (((1,), (1,)), ((), ()))
TN = (((0,), (0,)), ((), ()))


def _dot(a, b):
    return jnp.dot(a, b, preferred_element_type=F32)


def _dot_nt(a, b):
    return lax.dot_general(a, b, NT, preferred_element_type=F32)


def _dot_tn(a, b):
    return lax.dot_general(a, b, TN, preferred_element_type=F32)


def _layernorm(x):
    m = jnp.mean(x, axis=-1, keepdims=True)
    xc = x - m
    v = jnp.mean(xc * xc, axis=-1, keepdims=True)
    return xc * lax.rsqrt(v + LN_EPS)


U32 = jnp.uint32


def _pk(v):
    return pltpu.bitcast(v, U32)


def _upk(v):
    return pltpu.bitcast(v, BF)


def _recip(x):
    r = pl.reciprocal(x, approx=True)
    return r * (2.0 - x * r)


def _sub_reduce(a, op):
    a = op(a, pltpu.roll(a, 4, 0))
    return op(a, pltpu.roll(a, 2, 0))


def _phi(p):
    t = p.shape[-1]
    p3 = p.reshape(PR // 8, 8, t)
    mx = _sub_reduce(jnp.max(p3, axis=0), jnp.maximum)
    mn = _sub_reduce(jnp.min(p3, axis=0), jnp.minimum)
    ep = jnp.exp2(p3 - mx[None])
    en = jnp.exp2(mn[None] - p3)
    sp = _sub_reduce(jnp.sum(ep, axis=0), jnp.add)
    sn = _sub_reduce(jnp.sum(en, axis=0), jnp.add)
    phi = jnp.concatenate([ep * _recip(sp)[None], en * _recip(sn)[None]], axis=0)
    return phi.reshape(2 * PR, t).astype(BF)


def _kernel(x_hbm, wqkv_hbm, wphi_hbm, wo_hbm, w1_hbm, w3_hbm, w2_hbm, out_hbm,
            x_v, wqkv_v, wphi_v, wo_v, w1_v, w3_v, w2_v, obuf, xn_v,
            wkT, wvT, wqT, perm_v, a1, a2, bd_v, kv_acc, kv_bf, pq_v, hn_v, hres_v,
            wsem, osem):

    def x_copy(lo, hi, k):
        return pltpu.make_async_copy(x_hbm.at[0, pl.ds(lo, hi - lo)], x_v.at[pl.ds(lo, hi - lo)], wsem.at[9 + k])

    def w_copy(lo, hi, k):
        return pltpu.make_async_copy(wqkv_hbm.at[:, pl.ds(lo, hi - lo)], wqkv_v.at[:, pl.ds(lo, hi - lo)], wsem.at[k])

    cp_x0 = x_copy(0, T, 0)
    cp_x1 = x_copy(T, 2 * T, 1)
    cp_x2 = x_copy(2 * T, 3 * T, 2)
    cp_x3 = x_copy(3 * T, 4 * T, 6)
    cp_xs = x_copy(4 * T, S, 3)
    cp_k0 = w_copy(D, D + 128, 0)
    cp_k1 = w_copy(D + 128, D + 256, 1)
    cp_k2 = w_copy(D + 256, D + 512, 13)
    cp_k4 = w_copy(D + 512, 2 * D, 14)
    cp_v = w_copy(2 * D, 3 * D, 2)
    cp_q = w_copy(0, D, 8)
    cp_phi = pltpu.make_async_copy(wphi_hbm, wphi_v, wsem.at[3])
    cp_wo = pltpu.make_async_copy(wo_hbm, wo_v, wsem.at[4])
    cp_w1 = pltpu.make_async_copy(w1_hbm, w1_v, wsem.at[5])
    cp_w3 = pltpu.make_async_copy(w3_hbm, w3_v, wsem.at[6])
    cp_w2 = pltpu.make_async_copy(w2_hbm, w2_v, wsem.at[7])

    for cp in (cp_phi, cp_k0, cp_x0, cp_k1, cp_k2, cp_x1, cp_x2, cp_k4, cp_v, cp_x3, cp_xs, cp_q, cp_wo, cp_w1, cp_w3, cp_w2):
        cp.start()

    rp = lax.broadcasted_iota(jnp.int32, (16, 384), 0) * DH
    cp_ = lax.broadcasted_iota(jnp.int32, (16, 384), 1)
    dif = cp_ - rp
    zer = jnp.zeros((16, 256), BF)
    for d in range(DH):
        perm_v[pl.ds(d * H, 16), pl.ds(0, 384)] = jnp.where(dif == d, 1.0, 0.0).astype(BF)
        perm_v[pl.ds(d * H, 16), pl.ds(384, 256)] = zer
        perm_v[pl.ds(d * H + 16, 16), pl.ds(0, 256)] = zer
        perm_v[pl.ds(d * H + 16, 16), pl.ds(256, 384)] = jnp.where(dif == d + 16 * DH - 256, 1.0, 0.0).astype(BF)
    cp_phi.wait()
    for d in range(DH):
        a1[:, pl.ds(d * H, H)] = wphi_v[d].astype(F32)
    a1v = a1[...]
    for j in range(D // 128):
        a2[j, pl.ds(0, DH, stride=2), :] = a1v[:, j * 128:(j + 1) * 128]
        a2[j, pl.ds(1, DH, stride=2), :] = a1v[:, j * 128:(j + 1) * 128]
    a2v = jnp.concatenate([a2[j] for j in range(D // 128)], axis=1)
    a_full = _dot(a2v.astype(BF), perm_v[...])
    r2 = lax.broadcasted_iota(jnp.int32, (PR, 128), 0) & 1
    c2 = lax.broadcasted_iota(jnp.int32, (PR, 128), 1)
    for j in range(D // 128):
        blk = a_full[:, j * 128:(j + 1) * 128]
        parts = []
        for g in range(3 * j, 3 * j + 4):
            lo = (2 * g + r2) * DH - j * 128
            parts.append(jnp.where(jnp.logical_and(c2 >= lo, c2 < lo + DH), blk, 0.0))
        bd_v[j] = jnp.concatenate(parts, axis=0).astype(BF)

    def fold_blk(col0, j):
        return _dot_nt(bd_v[j], wqkv_v[:, pl.ds(col0 + j * 128, 128)])

    def emit(dst, row0, parts):
        rows = jnp.concatenate(parts, axis=0)
        dst[pl.ds(row0 // 2, rows.shape[0] // 2), :] = _pk((rows * LOG2E).astype(BF))

    def fold(dst, col0, j, prev):
        f = fold_blk(col0, j)
        head = [f[:PR]] if j == 0 else [prev[PC - PR:] + f[:PR]]
        if j % 2 == 1:
            head = [prev[112:PC - PR]] + head
        end = PC if j == 4 else (112 if j % 2 == 0 else PC - PR)
        emit(dst, j * (PC - PR) - (8 if j % 2 == 1 else 0), head + [f[PR:end]])
        return f

    def ln1(i, c):
        r0 = i * T + c * LC
        xn_v[pl.ds(r0 // 2, LC // 2), :] = _pk(_layernorm(x_v[pl.ds(r0, LC), :].astype(F32)).astype(BF))

    NLC = T // LC

    def proj(w, lo, n, i):
        return _dot_nt(_upk(w[pl.ds(lo // 2, n // 2), :]), _upk(xn_v[pl.ds(i * T // 2, T // 2), :]))

    ones8 = jnp.ones((8, T), F32)

    def vaug(v):
        return [jnp.concatenate([v[g * PR:(g + 1) * PR], ones8], axis=0).astype(BF) for g in range(v.shape[0] // PR)]

    def phis(p):
        return [_phi(p[g * PR:(g + 1) * PR]) for g in range(p.shape[0] // PR)]

    def kv_update(i, g0, vs, ps):
        for k, (v, p) in enumerate(zip(vs, ps)):
            r = _dot_nt(v, p)
            if i == 0:
                kv_acc[g0 + k] = r
            else:
                kv_acc[g0 + k] += r

    def qpiece(i, q):
        pq_v[i, pl.ds(q * PC, PC), :] = proj(wqT, q * PC, PC, i)

    def ln1_all(i):
        for c in range(NLC):
            ln1(i, c)

    cp_k0.wait()
    f = fold(wkT, D, 0, None)
    cp_x0.wait()
    ln1_all(0)
    cp_k1.wait()
    f = fold(wkT, D, 1, f)
    pk0 = [proj(wkT, 0, 112, 0), proj(wkT, 112, 128, 0)]
    cp_k2.wait()
    f = fold(wkT, D, 2, f)
    f = fold(wkT, D, 3, f)
    pk0.append(proj(wkT, 240, 112, 0))
    cp_x1.wait()
    pk0.append(proj(wkT, 352, 128, 0))
    ln1_all(1)
    pk1 = [proj(wkT, 0, PC, 1), proj(wkT, PC, PC, 1)]
    cp_x2.wait()
    cp_k4.wait()
    fold(wkT, D, 4, f)
    ln1_all(2)
    pk1.append(proj(wkT, 2 * PC, PC, 1))
    pk0.append(proj(wkT, 3 * PC, PC, 0))
    pk1.append(proj(wkT, 3 * PC, PC, 1))
    pk2 = [proj(wkT, 0, PC, 2), proj(wkT, PC, PC, 2)]
    cp_v.wait()
    cp_x3.wait()
    wvT[pl.ds(0, 128), :] = _pk(wqkv_v[:, pl.ds(2 * D, 256)].astype(F32).T.astype(BF))
    pk2.append(proj(wkT, 2 * PC, PC, 2))
    wvT[pl.ds(128, 192), :] = _pk(wqkv_v[:, pl.ds(2 * D + 256, 384)].astype(F32).T.astype(BF))
    pk2.append(proj(wkT, 3 * PC, PC, 2))
    pend = None
    for i, pk in enumerate((pk0, pk1, pk2)):
        pk = jnp.concatenate(pk, axis=0)
        for q in range(NPC):
            va = vaug(proj(wvT, q * PC, PC, i))
            if pend is not None:
                kv_update(*pend)
            pend = (i, 4 * q, va, phis(pk[q * PC:(q + 1) * PC]))
    ln1_all(3)

    qjobs = [(i, q) for i in range(NTILE) for q in range(NPC)]
    NHOLD = 6
    QB = 2
    for i in range(3, NTILE):
        for q in range(NPC):
            pk = proj(wkT, q * PC, PC, i)
            kv_update(*pend)
            if i == 3 and q == QB:
                cp_xs.wait()
                cp_q.wait()
                cp_wo.wait()
            if i + 1 < NTILE and (i > 3 or q >= QB):
                for c in (range(2 * q, 2 * q + 2) if i > 3 else range(4 * (q - QB), 4 * (q - QB) + 4)):
                    ln1(i + 1, c)
            va = vaug(proj(wvT, q * PC, PC, i))
            pend = (i, 4 * q, va, phis(pk))
            if i == 3 and q == QB:
                f = None
                for j in range(D // 128):
                    f = fold(wqT, 0, j, f)
            elif i > 3 or q > QB:
                for _ in range(2 if q % 2 == 0 else 1):
                    if len(qjobs) > NHOLD:
                        qpiece(*qjobs.pop(0))

    r3 = lax.broadcasted_iota(jnp.int32, (PA, 2 * PR), 0)
    c3 = lax.broadcasted_iota(jnp.int32, (PA, 2 * PR), 1) & 1
    hl3 = jnp.where(r3 < PR, jnp.where(r3 >= DH, 1, 0), jnp.where(r3 >= PR + 4, 1, 0))
    m3 = hl3 == c3
    low = lax.broadcasted_iota(jnp.int32, (8, T), 0) < 4

    def kv_fin(gs):
        for g in gs:
            kv_bf[g] = jnp.where(m3, kv_acc[g], 0.0).astype(BF)

    def num(g, ph):
        o = _dot(kv_bf[g], ph)
        r = _recip(o[PR:] + 1e-6)
        rs = pltpu.roll(r, 4, 0)
        r0 = jnp.where(low, r, rs)
        r1 = jnp.where(low, rs, r)
        return o[:PR] * jnp.concatenate([r0, r0, r, r1, r1], axis=0)

    def wo_res(oT, row0, slot):
        hres_v[slot] = x_v[pl.ds(row0, T), :].astype(F32) + _dot_tn(oT, wo_v[...])

    def ln2(slot, c):
        hn_v[pl.ds(c * LC // 2, LC // 2), :] = _pk(_layernorm(hres_v[slot, pl.ds(c * LC, LC), :]).astype(BF))

    NG = 6
    FH = F // NG
    GRP = (3, 3, 4, 3, 3, 0)

    def gateup(hn, c):
        gate = _dot(hn, w1_v[:, pl.ds(c * FH, FH)])
        up = _dot(hn, w3_v[:, pl.ds(c * FH, FH)])
        hg = 0.5 * gate
        return (hg * (1.0 + jnp.tanh(hg)) * up).astype(BF)

    def out_copy(k, lo, n):
        return pltpu.make_async_copy(obuf.at[pl.ds(lo, n)], out_hbm.at[0, pl.ds(lo, n)], osem.at[k])

    phq = phis(pq_v[0, pl.ds(0, 2 * PC), :])
    qpiece(*qjobs.pop(0))
    kv_fin(range(12))
    phq += phis(pq_v[0, pl.ds(2 * PC, 2 * PC), :])
    kv_update(*pend)
    o_parts = [num(g, phq[g]) for g in range(12)]
    kv_fin(range(12, 16))
    qpiece(*qjobs.pop(0))
    o_parts += [num(g, phq[g]) for g in range(12, 16)]
    qpiece(*qjobs.pop(0))
    wo_res(jnp.concatenate(o_parts, axis=0).astype(BF), 0, 0)
    while qjobs:
        qpiece(*qjobs.pop(0))
    for c in range(NLC):
        ln2(0, c)
    cp_w1.wait()
    cp_w3.wait()
    cp_w2.wait()

    def phase2(i, carry):
        row0 = pl.multiple_of(i * T, T)
        row1 = pl.multiple_of(row0 + T, T)
        slot = i % 2
        hn = _upk(hn_v[...])
        acts, o_parts = [], []
        for c in range(NG):
            acts.append(gateup(hn, c))
            for _ in range(GRP[c]):
                g = len(o_parts)
                o_parts.append(num(g, _phi(pq_v[i + 1, pl.ds(g * PR, PR), :])))
        wo_res(jnp.concatenate(o_parts, axis=0).astype(BF), row1, 1 - slot)
        act = jnp.concatenate(acts, axis=1)
        for n in range(D // 128):
            res = hres_v[slot, :, pl.ds(n * 128, 128)] + _dot(act, w2_v[:, pl.ds(n * 128, 128)])
            obuf[pl.ds(row0, T), pl.ds(n * 128, 128)] = res.astype(BF)
            for c in range(2 * n, min(2 * n + 2, NLC)):
                ln2(1 - slot, c)
        out_copy(i, row0, T).start()
        return carry

    lax.fori_loop(0, NTILE - 1, phase2, 0)
    last = NTILE - 1
    hn = _upk(hn_v[...])
    act = jnp.concatenate([gateup(hn, c) for c in range(NG)], axis=1)
    NW = D - 128
    r0 = last * T

    def tail_copy(k, lo, n, c0, nc):
        return pltpu.make_async_copy(obuf.at[pl.ds(r0 + lo, n), pl.ds(c0, nc)],
                                     out_hbm.at[0, pl.ds(r0 + lo, n), pl.ds(c0, nc)], osem.at[last + k])

    tail = ((0, T, 0, 384), (0, T, 384, 128), (0, 128, NW, 128), (128, 64, NW, 128), (192, 64, NW, 128))
    for k, (lo, n, c0, nc) in enumerate(tail):
        for c in range(c0, c0 + nc, 128):
            res = hres_v[last % 2, pl.ds(lo, n), pl.ds(c, 128)] + _dot(act[lo:lo + n], w2_v[:, pl.ds(c, 128)])
            obuf[pl.ds(r0 + lo, n), pl.ds(c, 128)] = res.astype(BF)
        tail_copy(k, lo, n, c0, nc).start()
    for i in range(NTILE - 1):
        out_copy(i, i * T, T).wait()
    for k, a in enumerate(tail):
        tail_copy(k, *a).wait()


@jax.jit
def pallas_sequential_preLN__linear_kernel_hedgehog__glu_gated_swiglu__prompt_kernel(
    A_x: jax.Array,
    A_wqkv: jax.Array,
    A_w_phi: jax.Array,
    A_wo: jax.Array,
    B_x: jax.Array,
    B_w1: jax.Array,
    B_w3: jax.Array,
    B_w2: jax.Array,
):
    any_spec = pl.BlockSpec(memory_space=pl.ANY)
    wphi_t = jnp.transpose(A_w_phi, (1, 2, 0))
    return pl.pallas_call(
        _kernel,
        out_shape=jax.ShapeDtypeStruct((1, S, D), BF),
        in_specs=[any_spec] * 7,
        out_specs=any_spec,
        scratch_shapes=[
            pltpu.VMEM((S, D), BF),
            pltpu.VMEM((D, 3 * D), BF),
            pltpu.VMEM((DH, DH, H), BF),
            pltpu.VMEM((D, D), BF),
            pltpu.VMEM((D, F), BF),
            pltpu.VMEM((D, F), BF),
            pltpu.VMEM((F, D), BF),
            pltpu.VMEM((S, D), BF),
            pltpu.VMEM((S // 2, D), U32),
            pltpu.VMEM((D // 2, D), U32),
            pltpu.VMEM((D // 2, D), U32),
            pltpu.VMEM((D // 2, D), U32),
            pltpu.VMEM((D, D), BF),
            pltpu.VMEM((DH, D), F32),
            pltpu.VMEM((D // 128, PR, 128), F32),
            pltpu.VMEM((D // 128, PC, 128), BF),
            pltpu.VMEM((NP, PA, 2 * PR), F32),
            pltpu.VMEM((NP, PA, 2 * PR), BF),
            pltpu.VMEM((NTILE, D, T), F32),
            pltpu.VMEM((T // 2, D), U32),
            pltpu.VMEM((2, T, D), F32),
            pltpu.SemaphoreType.DMA((16,)),
            pltpu.SemaphoreType.DMA((NTILE + 4,)),
        ],
        compiler_params=pltpu.CompilerParams(vmem_limit_bytes=100 * 1024 * 1024, disable_semaphore_checks=True),
    )(A_x, A_wqkv, wphi_t, A_wo, B_w1, B_w3, B_w2)
```

```python
import jax
import jax.numpy as jnp
from jax import lax
import jax.experimental.pallas as pl
import jax.experimental.pallas.tpu as pltpu

S, D, H, DH, F = 2048, 640, 32, 20, 1536
NP = H // 2
PR = 2 * DH
PA = PR + 8
PC = 4 * PR
NPC = D // PC
T = 256
NTILE = S // T
LC = 32
C0 = 256
NA, NB = 0, 4
LOG2E = 1.4426950408889634
LN_EPS = 1e-5
BF = jnp.bfloat16
F32 = jnp.float32

NT = (((1,), (1,)), ((), ()))
TN = (((0,), (0,)), ((), ()))


def _dot(a, b):
    return jnp.dot(a, b, preferred_element_type=F32)


def _dot_nt(a, b):
    return lax.dot_general(a, b, NT, preferred_element_type=F32)


def _dot_tn(a, b):
    return lax.dot_general(a, b, TN, preferred_element_type=F32)


def _layernorm(x):
    m = jnp.mean(x, axis=-1, keepdims=True)
    xc = x - m
    v = jnp.mean(xc * xc, axis=-1, keepdims=True)
    return xc * lax.rsqrt(v + LN_EPS)


U32 = jnp.uint32


def _pk(v):
    return pltpu.bitcast(v, U32)


def _upk(v):
    return pltpu.bitcast(v, BF)


def _recip(x):
    r = pl.reciprocal(x, approx=True)
    return r * (2.0 - x * r)


def _sub_reduce(a, op):
    a = op(a, pltpu.roll(a, 4, 0))
    return op(a, pltpu.roll(a, 2, 0))


def _phi(p):
    t = p.shape[-1]
    p3 = p.reshape(PR // 8, 8, t)
    mx = _sub_reduce(jnp.max(p3, axis=0), jnp.maximum)
    mn = _sub_reduce(jnp.min(p3, axis=0), jnp.minimum)
    ep = jnp.exp2(p3 - mx[None])
    en = jnp.exp2(mn[None] - p3)
    sp = _sub_reduce(jnp.sum(ep, axis=0), jnp.add)
    sn = _sub_reduce(jnp.sum(en, axis=0), jnp.add)
    phi = jnp.concatenate([ep * _recip(sp)[None], en * _recip(sn)[None]], axis=0)
    return phi.reshape(2 * PR, t).astype(BF)


def _kernel(x_hbm, wqkv_hbm, wphi_hbm, wo_hbm, w1_hbm, w3_hbm, w2_hbm, out_hbm,
            x_v, wqkv_v, wphi_v, wo_v, w1_v, w3_v, w2_v, obuf, xn_v,
            wkT, wvT, wqT, perm_v, a1, a2, bd_v, kv_acc, kv_bf, pq_v, hn_v, hres_v,
            wsem, bsem, osem):

    def x_copy(lo, hi, k):
        return pltpu.make_async_copy(x_hbm.at[0, pl.ds(lo, hi - lo)], x_v.at[pl.ds(lo, hi - lo)], wsem.at[9 + k])

    def w_copy(lo, hi, k):
        return pltpu.make_async_copy(wqkv_hbm.at[:, pl.ds(lo, hi - lo)], wqkv_v.at[:, pl.ds(lo, hi - lo)], wsem.at[k])

    cp_x0 = x_copy(0, T // 2, 0)
    cp_x0b = x_copy(T // 2, T, 7)
    cp_x1 = x_copy(T, 2 * T, 1)
    cp_x2 = x_copy(2 * T, 3 * T, 2)
    cp_x3 = x_copy(3 * T, 4 * T, 6)
    cp_xs = x_copy(4 * T, S, 3)
    cp_k0 = w_copy(D, D + 128, 0)
    cp_k1 = w_copy(D + 128, D + 256, 1)
    cp_k2 = w_copy(D + 256, D + 512, 13)
    cp_k4 = w_copy(D + 512, 2 * D, 14)
    cp_v = w_copy(2 * D, 3 * D, 2)
    cp_q = w_copy(0, D, 8)
    cp_phi = pltpu.make_async_copy(wphi_hbm, wphi_v, wsem.at[3])

    def blk_copies(src, dst, k0):
        return [pltpu.make_async_copy(src.at[:, pl.ds(n * 128, 128)], dst.at[n], bsem.at[k0 + n]) for n in range(dst.shape[0])]

    cp_wo = blk_copies(wo_hbm, wo_v, 0)
    cp_ffn = blk_copies(w1_hbm, w1_v, 5) + blk_copies(w3_hbm, w3_v, 17) + blk_copies(w2_hbm, w2_v, 29)
    w1_u, w3_u, w2_u, wo_u = (w.bitcast(U32) for w in (w1_v, w3_v, w2_v, wo_v))

    for cp in [cp_phi, cp_k0, cp_x0, cp_k1, cp_x0b, cp_k2, cp_x1, cp_x2, cp_k4, cp_v, cp_x3, cp_xs, cp_q] + cp_wo:
        cp.start()

    rp = lax.broadcasted_iota(jnp.int32, (16, 384), 0) * DH
    cp_ = lax.broadcasted_iota(jnp.int32, (16, 384), 1)
    dif = cp_ - rp
    zer = jnp.zeros((16, 256), BF)
    for d in range(DH):
        perm_v[pl.ds(d * H, 16), pl.ds(0, 384)] = jnp.where(dif == d, 1.0, 0.0).astype(BF)
        perm_v[pl.ds(d * H, 16), pl.ds(384, 256)] = zer
        perm_v[pl.ds(d * H + 16, 16), pl.ds(0, 256)] = zer
        perm_v[pl.ds(d * H + 16, 16), pl.ds(256, 384)] = jnp.where(dif == d + 16 * DH - 256, 1.0, 0.0).astype(BF)
    cp_phi.wait()
    for d in range(DH):
        a1[:, pl.ds(d * H, H)] = wphi_v[d].astype(F32)
    a1v = a1[...]
    for j in range(D // 128):
        a2[j, pl.ds(0, DH, stride=2), :] = a1v[:, j * 128:(j + 1) * 128]
        a2[j, pl.ds(1, DH, stride=2), :] = a1v[:, j * 128:(j + 1) * 128]
    a2v = jnp.concatenate([a2[j] for j in range(D // 128)], axis=1)
    a_full = _dot(a2v.astype(BF), perm_v[...])
    r2 = lax.broadcasted_iota(jnp.int32, (PR, 128), 0) & 1
    c2 = lax.broadcasted_iota(jnp.int32, (PR, 128), 1)
    for j in range(D // 128):
        blk = a_full[:, j * 128:(j + 1) * 128]
        parts = []
        for g in range(3 * j, 3 * j + 4):
            lo = (2 * g + r2) * DH - j * 128
            parts.append(jnp.where(jnp.logical_and(c2 >= lo, c2 < lo + DH), blk, 0.0))
        bd_v[j] = jnp.concatenate(parts, axis=0).astype(BF)

    def fold_blk(col0, j, split):
        w = wqkv_v[:, pl.ds(col0 + j * 128, 128)]
        if split:
            return jnp.concatenate([_dot_nt(bd_v[j, pl.ds(r, PC // 2), :], w) for r in (0, PC // 2)], axis=0)
        return _dot_nt(bd_v[j], w)

    def emit(dst, row0, parts):
        rows = jnp.concatenate(parts, axis=0)
        dst[pl.ds(row0 // 2, rows.shape[0] // 2), :] = _pk((rows * LOG2E).astype(BF))

    def fold(dst, col0, j, prev, split=False):
        f = fold_blk(col0, j, split)
        head = [f[:PR]] if j == 0 else [prev[PC - PR:] + f[:PR]]
        if j % 2 == 1:
            head = [prev[112:PC - PR]] + head
        end = PC if j == 4 else (112 if j % 2 == 0 else PC - PR)
        emit(dst, j * (PC - PR) - (8 if j % 2 == 1 else 0), head + [f[PR:end]])
        return f

    def ln1(i, c):
        r0 = i * T + c * LC
        xn_v[pl.ds(r0 // 2, LC // 2), :] = _pk(_layernorm(x_v[pl.ds(r0, LC), :].astype(F32)).astype(BF))

    NLC = T // LC

    def proj(w, lo, n, i, t0=0, nt=T):
        return _dot_nt(_upk(w[pl.ds(lo // 2, n // 2), :]), _upk(xn_v[pl.ds((i * T + t0) // 2, nt // 2), :]))

    ones8 = jnp.ones((8, T), F32)

    def vaug(v):
        return [jnp.concatenate([v[g * PR:(g + 1) * PR], ones8], axis=0).astype(BF) for g in range(v.shape[0] // PR)]

    def phis(p):
        return [_phi(p[g * PR:(g + 1) * PR]) for g in range(p.shape[0] // PR)]

    def kv_update(i, g0, vs, ps):
        for k, (v, p) in enumerate(zip(vs, ps)):
            r = _dot_nt(v, p)
            if i == 0:
                kv_acc[g0 + k] = r
            else:
                kv_acc[g0 + k] += r

    def qpiece(i, q, n=1):
        lo, n = int(q * PC), int(n * PC)
        pq_v[i, pl.ds(lo, n), :] = proj(wqT, lo, n, i)

    def ln1_all(i):
        for c in range(NLC):
            ln1(i, c)

    HT = T // 2
    cp_k0.wait()
    cp_x0.wait()
    f = fold(wkT, D, 0, None, True)
    for c in range(NLC // 2):
        ln1(0, c)
    cp_k1.wait()
    cp_x0b.wait()
    f = fold(wkT, D, 1, f, True)
    p0a = proj(wkT, 0, 112, 0, 0, HT)
    for c in range(NLC // 2, NLC):
        ln1(0, c)
    p0b = proj(wkT, 0, 112, 0, HT, HT)
    pk0 = [jnp.concatenate([p0a, p0b], axis=1), proj(wkT, 112, 128, 0)]
    cp_k2.wait()
    f = fold(wkT, D, 2, f)
    f = fold(wkT, D, 3, f, True)
    cp_x1.wait()
    pre = {}

    def prephi(i, pk, gs):
        pk = jnp.concatenate(pk, axis=0)
        for g in gs:
            pre[i, g] = _phi(pk[g * PR:(g + 1) * PR])

    prephi(0, pk0, range(NA))
    pk0.append(proj(wkT, 240, 112, 0))
    pk0.append(proj(wkT, 352, 128, 0))
    ln1_all(1)
    pk1 = [proj(wkT, 0, PC, 1), proj(wkT, PC, PC, 1)]
    cp_x2.wait()
    cp_k4.wait()
    fold(wkT, D, 4, f)
    prephi(0, pk0, range(NA, 12))
    prephi(1, pk1, range(NB))
    ln1_all(2)
    pk1.append(proj(wkT, 2 * PC, PC, 1))
    pk0.append(proj(wkT, 3 * PC, PC, 0))
    pk1.append(proj(wkT, 3 * PC, PC, 1))
    pk2 = [proj(wkT, 0, PC, 2), proj(wkT, PC, PC // 2, 2), proj(wkT, PC + PC // 2, PC // 2, 2)]
    cp_v.wait()
    cp_x3.wait()
    for cp in cp_ffn[:12]:
        cp.start()
    wvT[pl.ds(0, 128), :] = _pk(wqkv_v[:, pl.ds(2 * D, 256)].astype(F32).T.astype(BF))
    pk2.append(proj(wkT, 2 * PC, PC, 2))
    wvT[pl.ds(128, 192), :] = _pk(wqkv_v[:, pl.ds(2 * D + 256, 384)].astype(F32).T.astype(BF))
    pk2.append(proj(wkT, 3 * PC, PC, 2))
    pend = None
    for i, pk in enumerate((pk0, pk1, pk2)):
        pk = jnp.concatenate(pk, axis=0)
        for q in range(NPC):
            va = vaug(proj(wvT, q * PC, PC, i))
            if pend is not None:
                kv_update(*pend)
            pend = (i, 4 * q, va, [pre[i, g] if (i, g) in pre else _phi(pk[g * PR:(g + 1) * PR]) for g in range(4 * q, 4 * q + 4)])
    ln1_all(3)

    qdbl = [(i, q, 2) for i in (0, 1, 2, 5) for q in (0, 2)]
    qjobs = [(i, q) for i in (3, 4, 6) for q in range(NPC)] + [(7, 0, 2), (7, 2), (7, 3, 0.5), (7, 3.5, 0.5)]
    QB = 2
    for i in range(3, NTILE):
        for q in range(NPC):
            pk = proj(wkT, q * PC, PC, i)
            if i == 3 and q == QB:
                cp_xs.wait()
                cp_q.wait()
                for cp in cp_wo:
                    cp.wait()
                for cp in cp_ffn[12:]:
                    cp.start()
            kv_update(*pend)
            if i + 1 < NTILE and (i > 3 or q >= QB):
                for c in (range(2 * q, 2 * q + 2) if i > 3 else range(4 * (q - QB), 4 * (q - QB) + 4)):
                    ln1(i + 1, c)
            va = vaug(proj(wvT, q * PC, PC, i))
            pend = (i, 4 * q, va, phis(pk))
            if i == 3 and q == QB:
                f = None
                for j in range(D // 128):
                    f = fold(wqT, 0, j, f)
            elif i > 3 or q > QB:
                qpiece(*(qdbl if q % 2 == 0 else qjobs).pop(0))

    r3 = lax.broadcasted_iota(jnp.int32, (PA, 2 * PR), 0)
    c3 = lax.broadcasted_iota(jnp.int32, (PA, 2 * PR), 1) & 1
    hl3 = jnp.where(r3 < PR, jnp.where(r3 >= DH, 1, 0), jnp.where(r3 >= PR + 4, 1, 0))
    m3 = hl3 == c3
    low = lax.broadcasted_iota(jnp.int32, (8, T), 0) < 4

    def kv_fin(gs):
        for g in gs:
            kv_bf[g] = jnp.where(m3, kv_acc[g], 0.0).astype(BF)

    def num(g, ph):
        o = _dot(kv_bf[g], ph)
        r = _recip(o[PR:] + 1e-6)
        rs = pltpu.roll(r, 4, 0)
        r0 = jnp.where(low, r, rs)
        r1 = jnp.where(low, rs, r)
        return o[:PR] * jnp.concatenate([r0, r0, r, r1, r1], axis=0)

    def wo_res(oT, row0, slot):
        hres_v[slot] = x_v[pl.ds(row0, T), :].astype(F32) + _dot_tn(oT, jnp.concatenate([_upk(wo_u[n]) for n in range(D // 128)], axis=1))

    def ln2(slot, c):
        hn_v[pl.ds(c * LC // 2, LC // 2), :] = _pk(_layernorm(hres_v[slot, pl.ds(c * LC, LC), :]).astype(BF))

    NG = 6
    FH = F // NG
    GRP = (3, 3, 4, 3, 3, 0)

    def gateup(hn, c):
        gate = _dot(hn, jnp.concatenate([_upk(w1_u[2 * c]), _upk(w1_u[2 * c + 1])], axis=1))
        up = _dot(hn, jnp.concatenate([_upk(w3_u[2 * c]), _upk(w3_u[2 * c + 1])], axis=1))
        hg = 0.5 * gate
        return (hg * (1.0 + jnp.tanh(hg)) * up).astype(BF)

    NW = D - 128

    def out_copy(k, lo, n, c0=0, nc=NW):
        return pltpu.make_async_copy(obuf.at[pl.ds(lo, n), pl.ds(c0, nc)], out_hbm.at[0, pl.ds(lo, n), pl.ds(c0, nc)], osem.at[k])

    phq = phis(pq_v[0, pl.ds(0, 2 * PC), :])
    qpiece(*qjobs.pop(0))
    kv_fin(range(12))
    phq += phis(pq_v[0, pl.ds(2 * PC, 2 * PC), :])
    kv_update(*pend)
    o_parts = [num(g, phq[g]) for g in range(12)]
    kv_fin(range(12, 16))
    qpiece(*qjobs.pop(0))
    o_parts += [num(g, phq[g]) for g in range(12, 16)]
    qpiece(*qjobs.pop(0))
    wo_res(jnp.concatenate(o_parts, axis=0).astype(BF), 0, 0)
    while qjobs:
        qpiece(*qjobs.pop(0))
    for c in range(NLC):
        ln2(0, c)
    for cp in cp_ffn:
        cp.wait()

    def phase2(i, carry):
        row0 = pl.multiple_of(i * T, T)
        row1 = pl.multiple_of(row0 + T, T)
        slot = i % 2
        hn = _upk(hn_v[...])
        acts, o_parts = [], []
        for c in range(NG):
            acts.append(gateup(hn, c))
            for _ in range(GRP[c]):
                g = len(o_parts)
                o_parts.append(num(g, _phi(pq_v[i + 1, pl.ds(g * PR, PR), :])))
        wo_res(jnp.concatenate(o_parts, axis=0).astype(BF), row1, 1 - slot)
        act = jnp.concatenate(acts, axis=1)
        for n in range(D // 128):
            res = hres_v[slot, :, pl.ds(n * 128, 128)] + _dot(act, _upk(w2_u[n]))
            obuf[pl.ds(row0, T), pl.ds(n * 128, 128)] = res.astype(BF)
            for c in range(2 * n, min(2 * n + 2, NLC)):
                ln2(1 - slot, c)
        return carry

    lax.fori_loop(0, NTILE - 1, phase2, 0)
    last = NTILE - 1
    r0 = last * T
    cp_col = out_copy(0, 0, r0, 0, D)
    cp_col.start()
    hn = _upk(hn_v[...])
    act = jnp.concatenate([gateup(hn, c) for c in range(NG)], axis=1)

    def tail_copy(k, lo, n, c0, nc):
        return pltpu.make_async_copy(obuf.at[pl.ds(r0 + lo, n), pl.ds(c0, nc)],
                                     out_hbm.at[0, pl.ds(r0 + lo, n), pl.ds(c0, nc)], osem.at[1 + k])

    tail = ((0, T, 0, 384), (0, T, 384, 128), (0, 128, NW, 128), (128, 64, NW, 128), (192, 64, NW, 128))
    for k, (lo, n, c0, nc) in enumerate(tail):
        for c in range(c0, c0 + nc, 128):
            res = hres_v[last % 2, pl.ds(lo, n), pl.ds(c, 128)] + _dot(act[lo:lo + n], _upk(w2_u[c // 128]))
            obuf[pl.ds(r0 + lo, n), pl.ds(c, 128)] = res.astype(BF)
        tail_copy(k, lo, n, c0, nc).start()
    cp_col.wait()
    for k, a in enumerate(tail):
        tail_copy(k, *a).wait()


@jax.jit
def pallas_sequential_preLN__linear_kernel_hedgehog__glu_gated_swiglu__prompt_kernel(
    A_x: jax.Array,
    A_wqkv: jax.Array,
    A_w_phi: jax.Array,
    A_wo: jax.Array,
    B_x: jax.Array,
    B_w1: jax.Array,
    B_w3: jax.Array,
    B_w2: jax.Array,
):
    any_spec = pl.BlockSpec(memory_space=pl.ANY)
    wphi_t = jnp.transpose(A_w_phi, (1, 2, 0))
    return pl.pallas_call(
        _kernel,
        out_shape=jax.ShapeDtypeStruct((1, S, D), BF),
        in_specs=[any_spec] * 7,
        out_specs=any_spec,
        scratch_shapes=[
            pltpu.VMEM((S, D), BF),
            pltpu.VMEM((D, 3 * D), BF),
            pltpu.VMEM((DH, DH, H), BF),
            pltpu.VMEM((D // 128, D, 128), BF),
            pltpu.VMEM((F // 128, D, 128), BF),
            pltpu.VMEM((F // 128, D, 128), BF),
            pltpu.VMEM((D // 128, F, 128), BF),
            pltpu.VMEM((S, D), BF),
            pltpu.VMEM((S // 2, D), U32),
            pltpu.VMEM((D // 2, D), U32),
            pltpu.VMEM((D // 2, D), U32),
            pltpu.VMEM((D // 2, D), U32),
            pltpu.VMEM((D, D), BF),
            pltpu.VMEM((DH, D), F32),
            pltpu.VMEM((D // 128, PR, 128), F32),
            pltpu.VMEM((D // 128, PC, 128), BF),
            pltpu.VMEM((NP, PA, 2 * PR), F32),
            pltpu.VMEM((NP, PA, 2 * PR), BF),
            pltpu.VMEM((NTILE, D, T), F32),
            pltpu.VMEM((T // 2, D), U32),
            pltpu.VMEM((2, T, D), F32),
            pltpu.SemaphoreType.DMA((17,)),
            pltpu.SemaphoreType.DMA((34,)),
            pltpu.SemaphoreType.DMA((6,)),
        ],
        compiler_params=pltpu.CompilerParams(vmem_limit_bytes=100 * 1024 * 1024, disable_semaphore_checks=True),
    )(A_x, A_wqkv, wphi_t, A_wo, B_w1, B_w3, B_w2)
```

```python
import jax
import jax.numpy as jnp
from jax import lax
import jax.experimental.pallas as pl
import jax.experimental.pallas.tpu as pltpu

S, D, H, DH, F = 2048, 640, 32, 20, 1536
NP = H // 2
PR = 2 * DH
PA = PR + 8
PC = 4 * PR
NPC = D // PC
T = 256
NTILE = S // T
LC = 32
FB = 3 * PR
NFB = 6
NA, NB = 0, 8
CUT0 = (240, 320, 400, 480)
SPL = (0, 4)
ORP = "pqpunqNq"
Q7 = ((7, 0, 2), (7, 2), (7, 3, 0.5), (7, 3.5, 0.5))
OR6 = "t0p1T"
TS = 256
UB = 0
VC = ((0, 4, 8, 12, 16),) * 3
VO = (0, 1, 2)
VJ = [(i, a, b) for i in VO for a, b in zip(VC[i][:-1], VC[i][1:])]
ORD = "klmvpuq"
QD = (0, 1, 2, 5)
CUT1 = (0, 208, 416, 640)
CUT2 = (0, 320, 640)
CUT3 = (0, 128, 240)
CUT4 = (240, 448, 640)
PAT = ((2, 0, 2, 0), (2, 1, 0, 2), (1, 1, 0, 2), (1, 1, 0, 1), (2, 1, 0, 2), (0, 1, 0, 2))
LOG2E = 1.4426950408889634
LN_EPS = 1e-5
BF = jnp.bfloat16
F32 = jnp.float32

NT = (((1,), (1,)), ((), ()))
TN = (((0,), (0,)), ((), ()))


def _dot(a, b):
    return jnp.dot(a, b, preferred_element_type=F32)


def _dot_nt(a, b):
    return lax.dot_general(a, b, NT, preferred_element_type=F32)


def _dot_tn(a, b):
    return lax.dot_general(a, b, TN, preferred_element_type=F32)


def _layernorm(x):
    m = jnp.mean(x, axis=-1, keepdims=True)
    xc = x - m
    v = jnp.mean(xc * xc, axis=-1, keepdims=True)
    return xc * lax.rsqrt(v + LN_EPS)


U32 = jnp.uint32


def _pk(v):
    return pltpu.bitcast(v, U32)


def _upk(v):
    return pltpu.bitcast(v, BF)


def _recip(x):
    r = pl.reciprocal(x, approx=True)
    return r * (2.0 - x * r)


def _sub_reduce(a, op):
    a = op(a, pltpu.roll(a, 4, 0))
    return op(a, pltpu.roll(a, 2, 0))


def _phi(p):
    t = p.shape[-1]
    p3 = p.reshape(PR // 8, 8, t)
    mx = _sub_reduce(jnp.max(p3, axis=0), jnp.maximum)
    mn = _sub_reduce(jnp.min(p3, axis=0), jnp.minimum)
    ep = jnp.exp2(p3 - mx[None])
    en = jnp.exp2(mn[None] - p3)
    sp = _sub_reduce(jnp.sum(ep, axis=0), jnp.add)
    sn = _sub_reduce(jnp.sum(en, axis=0), jnp.add)
    phi = jnp.concatenate([ep * _recip(sp)[None], en * _recip(sn)[None]], axis=0)
    return phi.reshape(2 * PR, t).astype(BF)


def _kernel(x_hbm, wqkv_hbm, wphi_hbm, wo_hbm, w1_hbm, w3_hbm, w2_hbm, out_hbm,
            wqkv_v, x_v, wo_v, perm_v, w1_v, bd_v, w3_v, kv_acc, w2_v, obuf,
            pq_v, hn_v, hres_v, kv_bf, wphi_v, a1, a2, xn_v, wkT, wvT, wqT,
            wsem, bsem, osem):

    def x_copy(lo, hi, k):
        return pltpu.make_async_copy(x_hbm.at[0, pl.ds(lo, hi - lo)], x_v.at[pl.ds(lo, hi - lo)], wsem.at[9 + k])

    def w_copy(lo, hi, k):
        return pltpu.make_async_copy(wqkv_hbm.at[:, pl.ds(lo, hi - lo)], wqkv_v.at[:, pl.ds(lo, hi - lo)], wsem.at[k])

    cp_x0 = x_copy(0, T // 2, 0)
    cp_x0b = x_copy(T // 2, T, 7)
    cp_x1 = x_copy(T, 2 * T + T // 2, 1)
    cp_xs = x_copy(2 * T + T // 2, S, 3)
    cp_k0 = w_copy(D, D + 128, 0)
    cp_k1 = w_copy(D + 128, D + 256, 1)
    cp_k2 = w_copy(D + 256, D + 512, 13)
    cp_k4 = w_copy(D + 512, 2 * D, 14)
    cp_v = w_copy(2 * D, 3 * D, 2)
    cp_q = w_copy(0, D, 8)
    cp_phi = pltpu.make_async_copy(wphi_hbm, wphi_v, wsem.at[3])

    def blk_copies(src, dst, k0):
        return [pltpu.make_async_copy(src.at[:, pl.ds(n * 128, 128)], dst.at[n], bsem.at[k0 + n]) for n in range(dst.shape[0])]

    cp_wo = blk_copies(wo_hbm, wo_v, 0)
    cp_ffn = blk_copies(w1_hbm, w1_v, 5) + blk_copies(w3_hbm, w3_v, 17) + blk_copies(w2_hbm, w2_v, 29)
    w1_u, w3_u, w2_u, wo_u = (w.bitcast(U32) for w in (w1_v, w3_v, w2_v, wo_v))

    for cp in [cp_phi, cp_k0, cp_x0, cp_k1, cp_x0b, cp_k2]:
        cp.start()

    rp = lax.broadcasted_iota(jnp.int32, (16, 384), 0) * DH
    cp_ = lax.broadcasted_iota(jnp.int32, (16, 384), 1)
    dif = cp_ - rp
    zer = jnp.zeros((16, 256), BF)
    for d in range(DH):
        perm_v[pl.ds(d * H, 16), pl.ds(0, 384)] = jnp.where(dif == d, 1.0, 0.0).astype(BF)
        perm_v[pl.ds(d * H, 16), pl.ds(384, 256)] = zer
        perm_v[pl.ds(d * H + 16, 16), pl.ds(0, 256)] = zer
        perm_v[pl.ds(d * H + 16, 16), pl.ds(256, 384)] = jnp.where(dif == d + 16 * DH - 256, 1.0, 0.0).astype(BF)
    cp_phi.wait()
    for d in range(DH):
        a1[pl.ds(0, DH), pl.ds(d * H, H)] = wphi_v[d].astype(F32)
    a1v = a1[pl.ds(0, DH), :]
    for j in range(D // 128):
        a2[pl.ds(j * PR, DH, stride=2), :] = a1v[:, j * 128:(j + 1) * 128]
        a2[pl.ds(j * PR + 1, DH, stride=2), :] = a1v[:, j * 128:(j + 1) * 128]
    a2v = jnp.concatenate([a2[pl.ds(j * PR, PR), :] for j in range(D // 128)], axis=1)
    a_full = _dot(a2v.astype(BF), perm_v[pl.ds(0, D), :])
    r2 = lax.broadcasted_iota(jnp.int32, (PR, 128), 0) & 1
    c2 = lax.broadcasted_iota(jnp.int32, (PR, 128), 1)
    zer8 = jnp.zeros((8, 128), F32)

    def merge(j, get, lane):
        if j == 0 or j == NFB - 1:
            return get(min(j, NFB - 2))
        return jnp.where(lane >= 128 - 8 * j, get(j - 1), get(j))

    for j in range(NFB):
        blk = merge(j, lambda k: a_full[:, k * 128:(k + 1) * 128], c2)
        col = merge(j, lambda k: c2 + k * 128, c2)
        los = [(2 * g + r2) * DH for g in range(3 * j, min(3 * j + 3, NP))]
        parts = [jnp.where(jnp.logical_and(col >= lo, col < lo + DH), blk, 0.0) for lo in los]
        bd_v[pl.ds(j * 128, len(los) * PR + 8), :] = jnp.concatenate(parts + [zer8], axis=0).astype(BF)
    lane_w = lax.broadcasted_iota(jnp.int32, (D // 2, 128), 1)

    def emit(dst, row0, parts):
        rows = jnp.concatenate(parts, axis=0)
        dst[pl.ds(row0 // 2, rows.shape[0] // 2), :] = _pk((rows * LOG2E).astype(BF))

    def fold(dst, col0, j, prev, split=False):
        w = _upk(merge(j, lambda k: _pk(wqkv_v[:, pl.ds(col0 + k * 128, 128)]), lane_w))
        if j == NFB - 1:
            f = _dot_nt(bd_v[pl.ds(j * 128, PA), :], w)[:PR]
        elif split:
            f = jnp.concatenate([_dot_nt(bd_v[pl.ds(j * 128 + r, 64), :], w) for r in (0, 64)], axis=0)[:FB]
        else:
            f = _dot_nt(bd_v[pl.ds(j * 128, 128), :], w)[:FB]
        if j % 2 == 0:
            emit(dst, j * FB, [f[:FB - 8]])
        else:
            emit(dst, j * FB - 8, [prev[FB - 8:], f])
        return f

    def ln1(i, c):
        r0 = i * T + c * LC
        xn_v[pl.ds(r0 // 2, LC // 2), :] = _pk(_layernorm(x_v[pl.ds(r0, LC), :].astype(F32)).astype(BF))

    NLC = T // LC

    def proj(w, lo, n, i, t0=0, nt=T):
        return _dot_nt(_upk(w[pl.ds(lo // 2, n // 2), :]), _upk(xn_v[pl.ds((i * T + t0) // 2, nt // 2), :]))

    def vaug(v):
        ones8 = jnp.ones((8, v.shape[1]), F32)
        return [jnp.concatenate([v[g * PR:(g + 1) * PR], ones8], axis=0).astype(BF) for g in range(v.shape[0] // PR)]

    def phis(p):
        return [_phi(p[g * PR:(g + 1) * PR]) for g in range(p.shape[0] // PR)]

    def kv_update(i, g0, vs, ps):
        for k, (v, p) in enumerate(zip(vs, ps)):
            r = _dot_nt(v, p)
            if i == 0:
                kv_acc[pl.ds((g0 + k) * PA, PA), :] = r
            else:
                kv_acc[pl.ds((g0 + k) * PA, PA), :] += r

    def qpiece(i, q, n=1):
        lo, n = round(q * PC), round(n * PC)
        pq_v[i, pl.ds(lo, n), :] = proj(wqT, lo, n, i)

    def ln1_all(i):
        for c in range(NLC):
            ln1(i, c)

    HT = T // 2
    cp_k0.wait()
    cp_x0.wait()
    f = fold(wkT, D, 0, None, 0 in SPL)
    for c in range(NLC // 2):
        ln1(0, c)
    cp_k1.wait()
    cp_x0b.wait()
    for cp in [cp_k4, cp_x1]:
        cp.start()
    f = fold(wkT, D, 1, f, 1 in SPL)
    p0a = proj(wkT, 0, 112, 0, 0, HT)
    for c in range(NLC // 2, NLC):
        ln1(0, c)
    p0b = proj(wkT, 0, 112, 0, HT, HT)
    pk0 = [jnp.concatenate([p0a, p0b], axis=1), proj(wkT, 112, 128, 0)]
    cp_k2.wait()
    for cp in [cp_v]:
        cp.start()
    f = fold(wkT, D, 2, f, 2 in SPL)
    f = fold(wkT, D, 3, f, 3 in SPL)
    pk0 += [proj(wkT, lo, hi - lo, 0) for lo, hi in zip(CUT0[:-1], CUT0[1:])]
    cp_k4.wait()
    cp_x1.wait()
    for cp in [cp_xs, cp_q, *cp_wo]:
        cp.start()
    pre = {}

    def prephi(i, pk, gs):
        pk = jnp.concatenate(pk, axis=0)
        for g in gs:
            pre[i, g] = _phi(pk[g * PR:(g + 1) * PR])

    f = fold(wkT, D, 4, f, 4 in SPL)
    if CUT0[-1] < 480:
        pk0.append(proj(wkT, CUT0[-1], 480 - CUT0[-1], 0))
    fold(wkT, D, 5, f)
    pk0.append(proj(wkT, 480, PC, 0))

    def khalf(i, t0, cuts):
        for c in range(t0 // LC, (t0 + HT) // LC):
            ln1(i, c)
        return jnp.concatenate([proj(wkT, lo, hi - lo, i, t0, HT) for lo, hi in zip(cuts[:-1], cuts[1:])], axis=0)

    pk1 = [jnp.concatenate([khalf(1, 0, CUT1), khalf(1, HT, CUT2)], axis=1)]
    prephi(0, pk0, range(NA))
    pk2 = [khalf(2, 0, CUT3)]
    cp_v.wait()
    for cp in cp_ffn[:12]:
        cp.start()
    for op in OR6:
        if op == "t":
            wvT[pl.ds(0, TS // 2), :] = _pk(wqkv_v[:, pl.ds(2 * D, TS)].astype(F32).T.astype(BF))
        elif op == "T":
            wvT[pl.ds(TS // 2, (D - TS) // 2), :] = _pk(wqkv_v[:, pl.ds(2 * D + TS, D - TS)].astype(F32).T.astype(BF))
        elif op == "p":
            prephi(0, pk0, range(NA, NB))
        else:
            lo, hi = CUT4[int(op)], CUT4[int(op) + 1]
            pk2.append(proj(wkT, lo, hi - lo, 2, 0, HT))
    pend = None
    pks = [jnp.concatenate(pk, axis=0) for pk in (pk0, pk1, pk2)]
    for i, g0, g1 in VJ:
        pk = pks[i]
        if UB and pend is not None:
            kv_update(*pend)
        va = vaug(proj(wvT, g0 * PR, (g1 - g0) * PR, i, 0, pk.shape[1]))
        if not UB and pend is not None:
            kv_update(*pend)
        pend = (i, g0, va, [pre[i, g] if (i, g) in pre else _phi(pk[g * PR:(g + 1) * PR]) for g in range(g0, g1)])

    cp_xs.wait()
    cp_q.wait()
    for cp in cp_wo:
        cp.wait()
    for cp in cp_ffn[12:]:
        cp.start()
    kv_update(*pend)
    pend = None
    for c in range(NLC // 2, NLC):
        ln1(2, c)
    f = None
    for j in range(NFB):
        f = fold(wqT, 0, j, f)
    qdbl = [(i, q, 2) for i in QD for q in (0, 2)]
    qjobs = [(i, q) for i in range(7) if i not in QD for q in range(NPC)] + list(Q7)
    for i in range(2, NTILE):
        t0, nt = (HT, HT) if i == 2 else (0, T)
        for q in range(NPC):
            for op in ORD:
                if op == "k":
                    pk = proj(wkT, q * PC, PC, i, t0, nt)
                elif op == "u" and pend is not None:
                    kv_update(*pend)
                elif op in "lm" and i + 1 < NTILE:
                    ln1(i + 1, 2 * q + (op == "m"))
                elif op == "v":
                    va = vaug(proj(wvT, q * PC, PC, i, t0, nt))
                elif op == "p":
                    ph = phis(pk)
                elif op == "q" and PAT[i - 2][q]:
                    job = (qdbl if PAT[i - 2][q] == 2 else qjobs).pop(0)
                    assert job[0] <= i
                    qpiece(*job)
            pend = (i, 4 * q, va, ph)
    assert not qdbl and len(qjobs) >= 3

    r3 = lax.broadcasted_iota(jnp.int32, (PA, 2 * PR), 0)
    c3 = lax.broadcasted_iota(jnp.int32, (PA, 2 * PR), 1) & 1
    hl3 = jnp.where(r3 < PR, jnp.where(r3 >= DH, 1, 0), jnp.where(r3 >= PR + 4, 1, 0))
    m3 = hl3 == c3
    low = lax.broadcasted_iota(jnp.int32, (8, T), 0) < 4

    def kv_fin(gs):
        for g in gs:
            kv_bf[pl.ds(g * PA, PA), :] = jnp.where(m3, kv_acc[pl.ds(g * PA, PA), :], 0.0).astype(BF)

    def num(g, ph):
        o = _dot(kv_bf[pl.ds(g * PA, PA), :], ph)
        r = _recip(o[PR:] + 1e-6)
        rs = pltpu.roll(r, 4, 0)
        r0 = jnp.where(low, r, rs)
        r1 = jnp.where(low, rs, r)
        return o[:PR] * jnp.concatenate([r0, r0, r, r1, r1], axis=0)

    def wo_res(oT, row0, slot):
        hres_v[slot] = x_v[pl.ds(row0, T), :].astype(F32) + _dot_tn(oT, jnp.concatenate([_upk(wo_u[n]) for n in range(D // 128)], axis=1))

    def ln2(slot, c):
        hn_v[pl.ds(c * LC // 2, LC // 2), :] = _pk(_layernorm(hres_v[slot, pl.ds(c * LC, LC), :]).astype(BF))

    NG = 6
    FH = F // NG
    GRP = (3, 3, 4, 3, 3, 0)

    def gateup(hn, c):
        gate = _dot(hn, jnp.concatenate([_upk(w1_u[2 * c]), _upk(w1_u[2 * c + 1])], axis=1))
        up = _dot(hn, jnp.concatenate([_upk(w3_u[2 * c]), _upk(w3_u[2 * c + 1])], axis=1))
        hg = 0.5 * gate
        return (hg * (1.0 + jnp.tanh(hg)) * up).astype(BF)

    NW = D - 128

    def out_copy(k, lo, n, c0=0, nc=NW):
        return pltpu.make_async_copy(obuf.at[pl.ds(lo, n), pl.ds(c0, nc)], out_hbm.at[0, pl.ds(lo, n), pl.ds(c0, nc)], osem.at[k])

    phq, o_parts = [], []
    for op in ORP:
        if op == "p":
            phq += phis(pq_v[0, pl.ds(len(phq) * PR, 2 * PC), :])
        elif op == "q":
            qpiece(*qjobs.pop(0))
        elif op == "u":
            kv_update(*pend)
        elif op in "nN":
            gs = range(12) if op == "n" else range(12, 16)
            kv_fin(gs)
            o_parts += [num(g, phq[g]) for g in gs]
    assert ORP.index("u") < ORP.index("N") and len(o_parts) == NP
    wo_res(jnp.concatenate(o_parts, axis=0).astype(BF), 0, 0)
    while qjobs:
        qpiece(*qjobs.pop(0))
    for c in range(NLC):
        ln2(0, c)
    for cp in cp_ffn:
        cp.wait()

    def phase2(i, carry):
        row0 = pl.multiple_of(i * T, T)
        row1 = pl.multiple_of(row0 + T, T)
        slot = i % 2
        hn = _upk(hn_v[pl.ds(0, T // 2), :])
        acts, o_parts = [], []
        for c in range(NG):
            acts.append(gateup(hn, c))
            for _ in range(GRP[c]):
                g = len(o_parts)
                o_parts.append(num(g, _phi(pq_v[i + 1, pl.ds(g * PR, PR), :])))
        wo_res(jnp.concatenate(o_parts, axis=0).astype(BF), row1, 1 - slot)
        act = jnp.concatenate(acts, axis=1)
        for n in range(D // 128):
            res = hres_v[slot, :, pl.ds(n * 128, 128)] + _dot(act, _upk(w2_u[n]))
            obuf[pl.ds(row0, T), pl.ds(n * 128, 128)] = res.astype(BF)
            for c in range(2 * n, min(2 * n + 2, NLC)):
                ln2(1 - slot, c)
        return carry

    lax.fori_loop(0, NTILE - 1, phase2, 0)
    last = NTILE - 1
    r0 = last * T
    cp_col = out_copy(0, 0, r0, 0, D)
    cp_col.start()
    hn = _upk(hn_v[pl.ds(0, T // 2), :])
    act = jnp.concatenate([gateup(hn, c) for c in range(NG)], axis=1)

    def tail_copy(k, lo, n, c0, nc):
        return pltpu.make_async_copy(obuf.at[pl.ds(r0 + lo, n), pl.ds(c0, nc)],
                                     out_hbm.at[0, pl.ds(r0 + lo, n), pl.ds(c0, nc)], osem.at[1 + k])

    tail = ((0, T, 0, 384), (0, T, 384, 128), (0, 128, NW, 128), (128, 64, NW, 128), (192, 64, NW, 128))
    for k, (lo, n, c0, nc) in enumerate(tail):
        for c in range(c0, c0 + nc, 128):
            res = hres_v[last % 2, pl.ds(lo, n), pl.ds(c, 128)] + _dot(act[lo:lo + n], _upk(w2_u[c // 128]))
            obuf[pl.ds(r0 + lo, n), pl.ds(c, 128)] = res.astype(BF)
        tail_copy(k, lo, n, c0, nc).start()
    cp_col.wait()
    for k, a in enumerate(tail):
        tail_copy(k, *a).wait()


@jax.jit
def pallas_sequential_preLN__linear_kernel_hedgehog__glu_gated_swiglu__prompt_kernel(
    A_x: jax.Array,
    A_wqkv: jax.Array,
    A_w_phi: jax.Array,
    A_wo: jax.Array,
    B_x: jax.Array,
    B_w1: jax.Array,
    B_w3: jax.Array,
    B_w2: jax.Array,
):
    any_spec = pl.BlockSpec(memory_space=pl.ANY)
    wphi_t = jnp.transpose(A_w_phi, (1, 2, 0))
    return pl.pallas_call(
        _kernel,
        out_shape=jax.ShapeDtypeStruct((1, S, D), BF),
        in_specs=[any_spec] * 7,
        out_specs=any_spec,
        scratch_shapes=[
            pltpu.VMEM((D, 3 * D), BF),
            pltpu.VMEM((S, D), BF),
            pltpu.VMEM((D // 128, D, 128), BF),
            pltpu.VMEM((D, D), BF),
            pltpu.VMEM((F // 128, D, 128), BF),
            pltpu.VMEM((NFB * 128, 128), BF),
            pltpu.VMEM((F // 128, D, 128), BF),
            pltpu.VMEM((NP * PA, 2 * PR), F32),
            pltpu.VMEM((D // 128, F, 128), BF),
            pltpu.VMEM((S, D), BF),
            pltpu.VMEM((NTILE, D, T), F32),
            pltpu.VMEM((T // 2, D), U32),
            pltpu.VMEM((2, T, D), F32),
            pltpu.VMEM((NP * PA, 2 * PR), BF),
            pltpu.VMEM((DH, DH, H), BF),
            pltpu.VMEM((24, D), F32),
            pltpu.VMEM((D // 128 * PR, 128), F32),
            pltpu.VMEM((S // 2, D), U32),
            pltpu.VMEM((D // 2, D), U32),
            pltpu.VMEM((D // 2, D), U32),
            pltpu.VMEM((D // 2, D), U32),
            pltpu.SemaphoreType.DMA((17,)),
            pltpu.SemaphoreType.DMA((34,)),
            pltpu.SemaphoreType.DMA((6,)),
        ],
        compiler_params=pltpu.CompilerParams(vmem_limit_bytes=100 * 1024 * 1024, disable_semaphore_checks=True),
    )(A_x, A_wqkv, wphi_t, A_wo, B_w1, B_w3, B_w2)
```
